```python
import os as _os
_os.environ.setdefault("JAX_PLATFORMS", "cpu")
import jax
import jax.numpy as jnp

def _softmax(x, axis=-1):
    return jax.nn.softmax(x, axis=axis)
def _gelu(x):
    return jax.nn.gelu(x, approximate=True)
def _silu(x):
    return jax.nn.silu(x)
def _sigmoid(x):
    return jax.nn.sigmoid(x)
def _layernorm(x, axis=-1, eps=1e-5):
    m = jnp.mean(x, axis=axis, keepdims=True)
    v = jnp.var(x, axis=axis, keepdims=True)
    return (x - m) / jnp.sqrt(v + eps)
def _scatter_add(tgt, idx, src, axis=0):
    return tgt.at[idx].add(src)
def _segment_sum(src, seg, n):
    return jax.ops.segment_sum(src, seg, n)
class _Rng:
    def __init__(self, key):
        self._k = key
    def _next(self):
        self._k, sub = jax.random.split(self._k)
        return sub
    def normal(self, shape):
        return jax.random.normal(self._next(), shape, dtype=jnp.bfloat16)
    def randint(self, lo, hi, shape):
        return jax.random.randint(self._next(), shape, lo, hi, dtype=jnp.int32)
    def uniform(self, shape, lo=0.0, hi=1.0):
        return jax.random.uniform(self._next(), shape, jnp.bfloat16, lo, hi)
    def permutation(self, n):
        return jax.random.permutation(self._next(), n)


kernel_name = 'standalone__gqa_softmax__near_ridge'

def setup_inputs():
    _rng = _Rng(jax.random.key(int.from_bytes(__import__("os").urandom(4), "little")))
    _w = (lambda a: (lambda t: t.astype(jnp.bfloat16) if jnp.issubdtype(t.dtype, jnp.floating) else t)(jnp.asarray(a)))
    B, Hq, Hkv, Sq, Sk, D = 8, 32, 8, 112, 2048, 128
    return {
        "q": _w((lambda *s: _rng.normal(s) * 0.4)(B, Hq, Sq, D)),
        "k": _w((lambda *s: _rng.normal(s) * 0.4)(B, Hkv, Sk, D)),
        "v": _w((lambda *s: _rng.normal(s) * 0.05)(B, Hkv, Sk, D)),
    }

def reference(q, k, v):
    B, Hq, Sq, D = q.shape
    Hkv = k.shape[1]
    rep = Hq // Hkv
    k = jnp.repeat(k, rep, axis=1)
    v = jnp.repeat(v, rep, axis=1)
    scale = D ** -0.5
    scores = jnp.einsum("bhqd,bhkd->bhqk", q, k) * scale
    p = _softmax(scores, axis=-1)
    return jnp.einsum("bhqk,bhkd->bhqd", p, v)
```

```python
import jax
import jax.numpy as jnp
import numpy as np
from jax import lax
import jax.experimental.pallas as pl
import jax.experimental.pallas.tpu as pltpu

LOG2E = float(np.log2(np.e))
OPT = {'G': 2, 'CH': 512, 'PRESCALE': False, 'MUL': 'qk', 'LANCHOR': True, 'OANCHOR': True, 'WAITGRP': 2, 'BRANCH': True, 'ORDER': 'q0 q1 q2 e0 q3 p0 e1 p1 e2 p2 e3 p3', 'MLATE': True, 'MKEEP': False, 'OPAQUE': True, 'ROT': 0, 'COMB': False, 'INL': True, 'NOBC': True, 'BITCAST': True, 'FLAGS': {}}
G = OPT["G"]; CH = OPT["CH"]

@jax.jit
def pallas_standalone__gqa_softmax__near_ridge_kernel(q, k, v):
    B, Hq, Sq, D = q.shape
    _, Hkv, Sk, _ = k.shape
    rep = Hq // Hkv
    M = rep * Sq
    NP = B * Hkv
    NC = Sk // CH
    NIT = NP // G
    NT = CH // 128
    c = float(D ** -0.5) * LOG2E
    q3 = q.reshape(NP, M, D)
    k3 = k.reshape(NP, Sk, D)
    v3 = v.reshape(NP, Sk, D)

    def body(q_hbm, k_hbm, v_hbm, o_hbm, qbuf, kbuf, vbuf, obuf, s0, s1, m0, m1, mp_scr, z_ref, qs, ks, vs, os_):
        s_scr = (s0, s1); m_scr = (m0, m1)
        ZZ = [0, 0]
        def q_cp(p, slot):
            return pltpu.make_async_copy(q_hbm.at[p], qbuf.at[slot], qs.at[slot])
        def k_cp(p, slot):
            return pltpu.make_async_copy(k_hbm.at[p], kbuf.at[slot], ks.at[slot])
        def v_cp(p, slot):
            return pltpu.make_async_copy(v_hbm.at[p], vbuf.at[slot], vs.at[slot])
        def o_cp(p, slot):
            return pltpu.make_async_copy(obuf.at[slot], o_hbm.at[p], os_.at[slot])
        def fold(x, op):
            xs = [x[:, i * 128:(i + 1) * 128] for i in range(NT)]
            while len(xs) > 1:
                xs = [op(xs[i], xs[i + 1]) for i in range(0, len(xs), 2)]
            return xs[0]
        def rep_(m):
            return jnp.concatenate([m] * NT, axis=1) if NT > 1 else m

        def ld(buf, slot, r0, nr):
            if OPT["BITCAST"]:
                x = buf.bitcast(jnp.uint32)[slot, pl.ds(r0 // 2, nr // 2), :]
                return pltpu.bitcast(x, jnp.bfloat16)
            return buf[slot, pl.ds(r0, nr), :]
        def load_q(slot):
            qv = ld(qbuf, slot, 0, M)
            if OPT["PRESCALE"]:
                qv = (qv.astype(jnp.float32) * c).astype(jnp.bfloat16)
            return qv

        def qk_chunk(qv, slot, sslot, j, m):
            s = lax.dot_general(qv, ld(kbuf, slot, j * CH, CH), (((1,), (1,)), ((), ())),
                                preferred_element_type=jnp.float32)
            if OPT["MUL"] == "qk":
                s = s * c
            s_scr[sslot][ZZ[0], :, pl.ds(j * CH, CH)] = s
            mj = fold(s, jnp.maximum)
            m = mj if m is None else jnp.maximum(m, mj)
            if j == NC - 1:
                if OPT["MLATE"]:
                    m_scr[sslot][ZZ[0]] = m
                else:
                    mm = jnp.max(m, axis=-1, keepdims=True)
                    m_scr[sslot][ZZ[0]] = jnp.broadcast_to(mm, (M, 128))
            return m

        def e_chunk(sslot, j, st):
            l, o, m, P = st
            if m is None:
                m = m_scr[sslot][ZZ[1]]
                if OPT["MLATE"]:
                    m = jnp.broadcast_to(jnp.max(m, axis=-1, keepdims=True), (M, 128))
            m0_ = m
            if OPT["COMB"] and l is not None and o is not None:
                m = m + (l + o) * 0.0
            else:
                if OPT["LANCHOR"] and l is not None:
                    m = m + l * 0.0
                if OPT["OANCHOR"] and o is not None:
                    m = m + o * 0.0
            s = s_scr[sslot][ZZ[1], :, pl.ds(j * CH, CH)]
            x = s - rep_(m)
            if OPT["MUL"] == "sm":
                x = x * c
            p = jnp.exp2(x)
            lj = fold(p, jnp.add)
            l = lj if l is None else l + lj
            P[j] = p.astype(jnp.bfloat16)
            return l, o, (m0_ if (OPT['MLATE'] or OPT['MKEEP']) else None), P

        def p_chunk(slot, j, st):
            l, o, m, P = st
            oj = jnp.dot(P.pop(j), ld(vbuf, slot, j * CH, CH), preferred_element_type=jnp.float32)
            o = oj if o is None else o + oj
            if j == NC - 1:
                ll = jnp.sum(l, axis=-1, keepdims=True)
                obuf[slot] = (o * (1.0 / ll)).astype(obuf.dtype)
            return l, o, m, P

        def start_group(it, half):
            for t in range(G):
                p = it * G + t
                slot = half * G + t
                v_cp(p, slot).start()
                pn = jnp.minimum(p + 1, NP - 1)
                q_cp(pn, slot).start(); k_cp(pn, slot).start()

        z_ref[0] = 0; z_ref[1] = 0
        q_cp(0, 2 * G - 1).start(); k_cp(0, 2 * G - 1).start()
        start_group(0, 0)
        q_cp(0, 2 * G - 1).wait(); k_cp(0, 2 * G - 1).wait()
        m = None
        qv = load_q(2 * G - 1)
        for j in range(NC):
            m = qk_chunk(qv, 2 * G - 1, 0, j, m)

        if OPT["ROT"] > 0:
            q_cp(0, 0).wait(); k_cp(0, 0).wait()
            m = None
            qv = load_q(0)
            for j in range(OPT["ROT"]):
                m = qk_chunk(qv, 0, 1, j, m)
            mp_scr[...] = m

        def loop(it, carry, last=False, first=False):
            half = (it % 2) if (last or first) else lax.rem(it, 2)
            if last or first:
                ZZ[0] = ZV[0]; ZZ[1] = ZV[1]
            elif OPT['OPAQUE']:
                ZZ[0] = lax.div(it, 1 << 20); ZZ[1] = lax.div(it, 1 << 21)
            if not OPT["INL"]:
                @pl.when(it + 1 < NIT)
                def _():
                    start_group(it + 1, 1 - half)
            @pl.when(it >= 2) if not first else (lambda f: None)
            def _():
                for t in range(G):
                    o_cp((it - 2) * G + t, half * G + t).wait()
            R = OPT["ROT"]; W = 1 if first else OPT["WAITGRP"]
            def kslot(t):
                return half * G + t if t < G else (1 - half) * G
            m = mp_scr[...] if R > 0 else None
            for t0 in range(0, G, W):
                def waits(t0=t0):
                    for t in range(t0, t0 + W):
                        v_cp(0, half * G + t).wait()
                        tk = t + 1 if R > 0 else t
                        if tk < G:
                            q_cp(0, kslot(tk)).wait(); k_cp(0, kslot(tk)).wait()
                pl.when(it >= 0)(waits)
                if R > 0 and t0 + W == G:
                    @pl.when(it + 1 < NIT)
                    def _():
                        q_cp(0, kslot(G)).wait(); k_cp(0, kslot(G)).wait()
                for t in range(t0, t0 + W):
                    p = it * G + t
                    slot = half * G + t
                    st = (None, None, None, {})
                    if OPT["INL"] and not last:
                        pp = jnp.minimum(p + G, NP - 1); pn = jnp.minimum(p + G + 1, NP - 1); ns = (1 - half) * G + t
                        v_cp(pp, ns).start(); q_cp(pn, ns).start(); k_cp(pn, ns).start()
                    qv = load_q(slot)
                    for tok in OPT["ORDER"].split():
                        j = int(tok[1:])
                        if tok[0] == "q":
                            if j >= R and not (last and t == G - 1):
                                m = qk_chunk(qv, slot, (t + 1) % 2, j, m)
                                if j == NC - 1: m = None
                        else:
                            if tok[0] in "se": st = e_chunk(t % 2, j, st)
                            if tok[0] in "sp": st = p_chunk(slot, j, st)
                    o_cp(p, slot).start()
                    if R > 0:
                        qv = load_q(kslot(t + 1))
                        for j in range(R):
                            m = qk_chunk(qv, kslot(t + 1), t % 2, j, m)
            if R > 0:
                mp_scr[...] = m
            return carry
        ZV = [z_ref[0], z_ref[1]]
        loop(0, 0, first=True)
        lax.fori_loop(1, NIT - 1, loop, 0)
        loop(NIT - 1, 0, last=True)
        for t in range(2 * G):
            o_cp(NP - 2 * G + t, ((NIT - 2) % 2 * G + t) % (2 * G)).wait()

    out = pl.pallas_call(
        body,
        in_specs=[pl.BlockSpec(memory_space=pl.ANY)] * 3,
        out_specs=pl.BlockSpec(memory_space=pl.ANY),
        out_shape=jax.ShapeDtypeStruct((NP, M, D), q.dtype),
        scratch_shapes=[
            pltpu.VMEM((2 * G, M, D), q.dtype), pltpu.VMEM((2 * G, Sk, D), k.dtype), pltpu.VMEM((2 * G, Sk, D), v.dtype),
            pltpu.VMEM((2 * G, M, D), q.dtype), pltpu.VMEM((1, M, Sk), jnp.float32), pltpu.VMEM((1, M, Sk), jnp.float32),
            pltpu.VMEM((1, M, 128), jnp.float32), pltpu.VMEM((1, M, 128), jnp.float32), pltpu.VMEM((M, 128), jnp.float32), pltpu.SMEM((2,), jnp.int32),
            pltpu.SemaphoreType.DMA((2 * G,)), pltpu.SemaphoreType.DMA((2 * G,)), pltpu.SemaphoreType.DMA((2 * G,)),
            pltpu.SemaphoreType.DMA((2 * G,)),
        ],
        compiler_params=pltpu.CompilerParams(vmem_limit_bytes=100 * 1024 * 1024, flags=OPT["FLAGS"], disable_bounds_checks=OPT["NOBC"]),
    )(q3, k3, v3)
    return out.reshape(B, Hq, Sq, D)
```
